```python
import jax
import jax.numpy as jnp

def _softmax(x, axis=-1):
    return jax.nn.softmax(x, axis=axis)
def _gelu(x):
    return jax.nn.gelu(x, approximate=True)
def _silu(x):
    return jax.nn.silu(x)
def _sigmoid(x):
    return jax.nn.sigmoid(x)
def _layernorm(x, axis=-1, eps=1e-5):
    m = jnp.mean(x, axis=axis, keepdims=True)
    v = jnp.var(x, axis=axis, keepdims=True)
    return (x - m) / jnp.sqrt(v + eps)
def _scatter_add(tgt, idx, src, axis=0):
    return tgt.at[idx].add(src)
def _segment_sum(src, seg, n):
    return jax.ops.segment_sum(src, seg, n)
class _Rng:
    def __init__(self, key):
        self._k = key
    def _next(self):
        self._k, sub = jax.random.split(self._k)
        return sub
    def normal(self, shape):
        return jax.random.normal(self._next(), shape, dtype=jnp.bfloat16)
    def randint(self, lo, hi, shape):
        return jax.random.randint(self._next(), shape, lo, hi, dtype=jnp.int32)
    def uniform(self, shape, lo=0.0, hi=1.0):
        return jax.random.uniform(self._next(), shape, jnp.bfloat16, lo, hi)
    def permutation(self, n):
        return jax.random.permutation(self._next(), n)


kernel_name = 'parallel_sum__linear_kernel_hedgehog__glu_gated_bilinear__prompt'

def _fwd_setup_inputs():
    _rng = _Rng(jax.random.key(int.from_bytes(__import__("os").urandom(4), "little")))
    _w = (lambda a: (lambda t: t.astype(jnp.bfloat16) if jnp.issubdtype(t.dtype, jnp.floating) else t)(jnp.asarray(a)))
    def _A_setup():
        B, S, D, H = 1, 2048, 512, 32
        Dh = D // H
        return {
            "x": _w((lambda *s: _rng.normal(s) * 0.05)(B, S, D)),
            "wqkv": _w((lambda *s: _rng.normal(s) * 0.05)(D, 3 * D)),
            "w_phi": _w((lambda *s: _rng.normal(s) * 0.05)(H, Dh, Dh) * (Dh ** -0.5)),
            "wo": _w((lambda *s: _rng.normal(s) * 0.05)(D, D)),
        }
    _A_in = _A_setup()

    def _B_setup():
        B, S, D, F = 1, 2048, 512, 1792
        return {
            "x": _w((lambda *s: _rng.normal(s) * 0.05)(B, S, D)),
            "w_gate": _w((lambda *s: _rng.normal(s) * 0.05)(D, F) * (D ** -0.5)),
            "w_up": _w((lambda *s: _rng.normal(s) * 0.05)(D, F) * (D ** -0.5)),
            "w_down": _w((lambda *s: _rng.normal(s) * 0.05)(F, D) * (F ** -0.5)),
        }
    _B_in = _B_setup()

    return {
        "A_x": _A_in["x"],
        "A_wqkv": _A_in["wqkv"],
        "A_w_phi": _A_in["w_phi"],
        "A_wo": _A_in["wo"],
        "B_x": _B_in["x"],
        "B_w_gate": _B_in["w_gate"],
        "B_w_up": _B_in["w_up"],
        "B_w_down": _B_in["w_down"],
    }

def _fwd_reference(A_x, A_wqkv, A_w_phi, A_wo, B_x, B_w_gate, B_w_up, B_w_down):
    def _A_ref(x, wqkv, w_phi, wo):
        B, S, D = x.shape
        H = 32; Dh = D // H
        qkv = (lambda x, *d: x.transpose(*d))((x @ wqkv).reshape(B, S, 3, H, Dh), 2, 0, 3, 1, 4)
        q, k, v = qkv[0], qkv[1], qkv[2]
        pq = jnp.einsum("bhsd,hdf->bhsf", q, w_phi)
        pk = jnp.einsum("bhsd,hdf->bhsf", k, w_phi)
        phi_q = jnp.concatenate([_softmax(pq, axis=-1), _softmax(-pq, axis=-1)], axis=-1)
        phi_k = jnp.concatenate([_softmax(pk, axis=-1), _softmax(-pk, axis=-1)], axis=-1)
        kv = jnp.einsum("bhsf,bhsd->bhfd", phi_k, v)
        z  = jnp.einsum("bhsf->bhf", phi_k)
        num = jnp.einsum("bhqf,bhfd->bhqd", phi_q, kv)
        den = jnp.einsum("bhqf,bhf->bhq", phi_q, z)[..., None] + 1e-6
        o = num / den
        return (lambda x, *d: x.transpose(*d))(o, 0, 2, 1, 3).reshape(B, S, D) @ wo

    def _B_ref(x, w_gate, w_up, w_down):
        g = jnp.einsum("bsd,df->bsf", x, w_gate)
        u = jnp.einsum("bsd,df->bsf", x, w_up)
        h = g * u
        return jnp.einsum("bsf,fd->bsd", h, w_down)

    x = A_x
    xn = _layernorm(x, axis=-1)
    return x + _A_ref(xn, A_wqkv, A_w_phi, A_wo) + _B_ref(xn, B_w_gate, B_w_up, B_w_down)


def setup_inputs():
    _inp = _fwd_setup_inputs()
    _gk = jax.random.fold_in(jax.random.key(int.from_bytes(__import__("os").urandom(4), "little")), 2**31 - 1)
    _shapes = [[1, 2048, 512]]
    _dtypes = ['bfloat16']
    _gks = jax.random.split(_gk, len(_shapes))
    _gs = [jax.random.normal(k, s, dtype=jnp.dtype(d)) * 0.05 for k, s, d in zip(_gks, _shapes, _dtypes)]
    _inp["grad_out"] = _gs[0]
    return _inp

def reference(A_x, A_wqkv, A_w_phi, A_wo, B_w_gate, B_w_up, B_w_down, B_x, grad_out):
    _const = dict(B_x=B_x)
    def _f(*_d):
        return _fwd_reference(**{'A_x': _d[0], 'A_wqkv': _d[1], 'A_w_phi': _d[2], 'A_wo': _d[3], 'B_w_gate': _d[4], 'B_w_up': _d[5], 'B_w_down': _d[6], **_const})
    _out, _vjp = jax.vjp(_f, A_x, A_wqkv, A_w_phi, A_wo, B_w_gate, B_w_up, B_w_down)
    _grads = _vjp(grad_out)
    _out0 = jnp.asarray(_out)
    return (_out0, *[jnp.asarray(_g) for _g in _grads])
```

```python
import jax
import jax.numpy as jnp
import jax.experimental.pallas as pl
import jax.experimental.pallas.tpu as pltpu

F32 = jnp.float32
BF16 = jnp.bfloat16

S = 2048
D = 512
H = 32
DH = 16
FF = 1792
NG = 4
TS = 256
NTL = S // TS
FC = 256
NFC = FF // FC
RP = D // NTL
LN_EPS = 1e-5
DEN_EPS = 1e-6


def _nn(a, b):
    return jnp.dot(a, b, preferred_element_type=F32)


def _nt(a, b):
    return jax.lax.dot_general(a, b, (((1,), (1,)), ((), ())), preferred_element_type=F32)


def _tn(a, b):
    return jax.lax.dot_general(a, b, (((0,), (0,)), ((), ())), preferred_element_type=F32)


def _iota(shape, dim):
    return jax.lax.broadcasted_iota(jnp.int32, shape, dim)


def _onehot(cond):
    return jnp.where(cond, 1.0, 0.0).astype(BF16)


def _dual_softmax(p):
    t = p.shape[-1]
    p3 = p.reshape(DH, 8, t)
    mx = jnp.max(p3, axis=0)
    mn = jnp.min(p3, axis=0)
    ep = jnp.exp(p3 - mx[None])
    em = jnp.exp(mn[None] - p3)
    rp = 1.0 / jnp.sum(ep, axis=0)
    rm = 1.0 / jnp.sum(em, axis=0)
    return ep * rp[None], em * rm[None]


def _dual_softmax_bwd(php, phm, dphp, dphm):
    tp = jnp.sum(dphp * php, axis=0)
    tm = jnp.sum(dphm * phm, axis=0)
    dp = php * (dphp - tp[None]) - phm * (dphm - tm[None])
    return dp.reshape(128, dp.shape[-1])


def _lane_fold(a):
    t = a.shape[-1]
    acc = a[:, 0:128]
    for j in range(1, t // 128):
        acc = acc + a[:, j * 128:(j + 1) * 128]
    return acc


def _perm_mats():
    r = _iota((128, 128), 0)
    c = _iota((128, 128), 1)
    pi = _onehot((r // 8 == c % 16) & (r % 8 == c // 16))
    pit = _onehot((c // 8 == r % 16) & (c % 8 == r // 16))
    return pi, pit


def _wphi_mats():
    h = _iota((H, D), 0)
    j = _iota((H, D), 1)
    sel = _onehot(h == (j // 128) * 8 + j % 8)
    a = _iota((256, D), 0)
    j2 = _iota((256, D), 1)
    fmask = a % 16 == (j2 % 128) // 8
    c = _iota((128, 256), 0)
    a2 = _iota((128, 256), 1)
    rep = _onehot(c % 16 == a2 // 16)
    c3 = _iota((128, D), 0)
    j3 = _iota((128, D), 1)
    hmask = c3 // 16 == j3 % 8
    return sel, fmask, rep, hmask


def _head_mask():
    r = _iota((256, 128), 0)
    c = _iota((256, 128), 1)
    return r % 8 == c % 8


def _kernel(x_hbm, dy_hbm, wqkv_hbm, wphi_hbm, wo_hbm, wg_hbm, wu_hbm, wd_hbm,
            out_hbm, dx_hbm, dwqkv_hbm, dwphi_hbm, dwo_hbm, dwg_hbm, dwu_hbm, dwd_hbm,
            x_v, dy_v, wqkv_v, wphi_v, wo_v, wgu_v, wd_v,
            wT, wN, wop, PT_s, dP_s,
            xn_s, xnT_s, phik_s, vT_s, dpT_s, pq_s, doT_s,
            kv_acc, z_acc, dkv_acc, dz_acc,
            kvm_s, kvtz_s, zb_s,
            h_s, dgu_s,
            g_acc, dwo_acc, dwgu_acc, dwdT_acc,
            o_out, o_dx, o_dwqkv, o_dwphi, o_dwo, o_dwg, o_dwu, o_dwd,
            sem_x, sem_dy, sem_w, sem_o, sem_dx, sem_dw, sem_g, sem_u, sem_d):

    def tile(i):
        return pl.ds(pl.multiple_of(i * TS, TS), TS)

    def cp_x(i):
        return pltpu.make_async_copy(x_hbm.at[tile(i), :], x_v.at[tile(i), :], sem_x.at[i])

    def cp_dy(i):
        return pltpu.make_async_copy(dy_hbm.at[tile(i), :], dy_v.at[tile(i), :], sem_dy.at[i])

    def cp_out(i):
        return pltpu.make_async_copy(o_out.at[tile(i), :], out_hbm.at[tile(i), :], sem_o.at[i])

    def cp_dx(i):
        return pltpu.make_async_copy(o_dx.at[tile(i), :], dx_hbm.at[tile(i), :], sem_dx.at[i])

    def piece(i):
        return pl.ds(pl.multiple_of(i * RP, RP), RP)

    def cp_dwg(i):
        return pltpu.make_async_copy(o_dwg.at[piece(i), :], dwg_hbm.at[piece(i), :], sem_g.at[i])

    def cp_dwu(i):
        return pltpu.make_async_copy(o_dwu.at[piece(i), :], dwu_hbm.at[piece(i), :], sem_u.at[i])

    def cp_dwd(i):
        rows = pl.ds(pl.multiple_of(i * FC, FC), FC)
        return pltpu.make_async_copy(o_dwd.at[rows, :], dwd_hbm.at[rows, :], sem_d.at[i])

    def cp_wpart(part):
        cols = slice(part * D, (part + 1) * D)
        return pltpu.make_async_copy(wqkv_hbm.at[:, cols], wqkv_v.at[:, cols], sem_w.at[part])

    def cp_dwpart(part):
        cols = slice(part * D, (part + 1) * D)
        return pltpu.make_async_copy(o_dwqkv.at[:, cols], dwqkv_hbm.at[:, cols], sem_dw.at[part])

    cp_wphi = pltpu.make_async_copy(wphi_hbm, wphi_v, sem_w.at[3])
    cp_wo = pltpu.make_async_copy(wo_hbm, wo_v, sem_w.at[4])
    cp_wg = pltpu.make_async_copy(wg_hbm, wgu_v.at[:, 0:FF], sem_w.at[5])
    cp_wu = pltpu.make_async_copy(wu_hbm, wgu_v.at[:, FF:2 * FF], sem_w.at[6])
    cp_wd = pltpu.make_async_copy(wd_hbm, wd_v, sem_w.at[7])
    cp_dwphi = pltpu.make_async_copy(o_dwphi, dwphi_hbm, sem_dw.at[3])
    cp_dwo = pltpu.make_async_copy(o_dwo, dwo_hbm, sem_dw.at[4])

    def layernorm_tile(j):
        tok = tile(j)
        x = x_v[tok, :].astype(F32)
        mu = jnp.mean(x, axis=-1, keepdims=True)
        xc = x - mu
        var = jnp.mean(xc * xc, axis=-1, keepdims=True)
        xn32 = xc * jax.lax.rsqrt(var + LN_EPS)
        xn_s[tok, :] = xn32.astype(BF16)
        xnT_s[:, tok] = xn32.T.astype(BF16)

    with jax.named_scope("prologue"):
        cp_wphi.start()
        cp_x(0).start()
        cp_wpart(1).start()
        sel, fmask, rep, hmask = _wphi_mats()
        cp_wphi.wait()
        cp_wpart(2).start()
        a2 = wphi_v[...].reshape(DH * DH, H)
        b = jnp.where(fmask, _nn(a2, sel), 0.0).astype(BF16)
        p_all = jnp.where(hmask, _nn(rep, b), 0.0)
        for g in range(NG):
            PT_s[g * 128:(g + 1) * 128, :] = p_all[:, g * 128:(g + 1) * 128].T.astype(BF16)

        def prep(part):
            for g in range(NG):
                cols = slice(part * D + g * 128, part * D + (g + 1) * 128)
                wT[cols, :] = _nt(PT_s[g * 128:(g + 1) * 128, :], wqkv_v[:, cols]).astype(BF16)

        cp_x(0).wait()
        cp_wpart(0).start()
        cp_wpart(1).wait()
        cp_wo.start()
        cp_dy(0).start()
        prep(1)
        layernorm_tile(0)
        cp_wpart(2).wait()
        cp_wpart(0).wait()
        for i in range(1, NTL):
            cp_x(i).start()
            cp_dy(i).start()
        prep(0)
        wT[2 * D:3 * D, :] = wqkv_v[:, 2 * D:3 * D].astype(F32).T.astype(BF16)
        cp_wo.wait()
        cp_wd.start()
        cp_wg.start()
        cp_wu.start()
        pi, _ = _perm_mats()
        for g in range(NG):
            rows = slice(g * 128, (g + 1) * 128)
            wop[rows, :] = _nn(pi, wo_v[rows, :]).astype(BF16)

    def phase0(i, carry):
        tok = tile(i)

        @pl.when(i + 1 < NTL)
        def _():
            cp_x(i + 1).wait()

        cp_dy(i).wait()
        xn = xn_s[tok, :]
        phbs = {}

        def sm(g):
            pk = _nt(wT[D + g * 128:D + (g + 1) * 128, :], xn)
            php, phm = _dual_softmax(pk)
            ph = jnp.concatenate([php.reshape(128, TS), phm.reshape(128, TS)], axis=0)
            phb = ph.astype(BF16)
            phik_s[g * 256:(g + 1) * 256, tok] = phb
            z_acc[g * 256:(g + 1) * 256, :] = jnp.where(i > 0, z_acc[g * 256:(g + 1) * 256, :], 0.0) + _lane_fold(ph)
            phbs[g] = phb

        def pqm(g):
            pq_s[g * 128:(g + 1) * 128, tok] = _nt(wT[g * 128:(g + 1) * 128, :], xn)

        def kvm(g):
            kv_acc[g * 256:(g + 1) * 256, :] = (jnp.where(i > 0, kv_acc[g * 256:(g + 1) * 256, :], 0.0)
                                                + _nt(phbs[g], vT[g * 128:(g + 1) * 128, :]))

        sm(0); sm(1)
        vT = _nt(wT[2 * D:3 * D, :], xn).astype(BF16)
        vT_s[:, tok] = vT
        sm(2); kvm(0); kvm(1); pqm(0)
        sm(3); pqm(1); kvm(2); pqm(2); kvm(3)
        layernorm_tile(jnp.minimum(i + 1, NTL - 1))
        doT_s[:, tok] = _nt(wop[...], dy_v[tok, :])
        pqm(3)
        return carry

    with jax.named_scope("phase0"):
        jax.lax.fori_loop(0, NTL, phase0, 0)

    with jax.named_scope("prologue1"):
        r = _iota((256, 128), 0)
        c = _iota((256, 128), 1)
        _, pit = _perm_mats()
        for g in range(NG):
            rows = slice(g * 256, (g + 1) * 256)
            kvn = jnp.where(r % 8 == c // 16, kv_acc[rows, :], 0.0).astype(BF16)
            kvm = _nn(kvn, pit)
            zb = jnp.broadcast_to(jnp.sum(z_acc[rows, :], axis=-1, keepdims=True), (256, 128))
            zb_s[rows, :] = zb
            zc = jnp.where(c == r % 8, zb, 0.0)
            kvm_s[rows, :] = kvm.astype(BF16)
            both_t = jnp.concatenate([kvm, zc], axis=1).T
            kvtz_s[g * 144:(g + 1) * 144, :] = both_t[0:144, :].astype(BF16)
        cp_wd.wait()
        cp_wg.wait()
        cp_wu.wait()

    def phase1(i, carry):
        tok = tile(i)
        xn = xn_s[tok, :]
        xnT = xnT_s[:, tok]
        dy = dy_v[tok, :]
        st = {}

        def fa(c):
            st['gg', c] = _nn(xn, wgu_v[:, c * FC:(c + 1) * FC])

        def fb(c):
            uu = _nn(xn, wgu_v[:, FF + c * FC:FF + (c + 1) * FC])
            st['uu', c] = uu
            h_s[:, c * FC:(c + 1) * FC] = (st['gg', c] * uu).astype(BF16)

        def fc(c):
            dh = _nt(dy, wd_v[c * FC:(c + 1) * FC, :])
            dgu_s[tok, c * FC:(c + 1) * FC] = (dh * st['uu', c]).astype(BF16)
            dgu_s[tok, FF + c * FC:FF + (c + 1) * FC] = (dh * st['gg', c]).astype(BF16)

        def sm(g):
            php, phm = _dual_softmax(pq_s[g * 128:(g + 1) * 128, tok])
            ph = jnp.concatenate([php.reshape(128, TS), phm.reshape(128, TS)], axis=0)
            st['ph', g] = (php, phm, ph, ph.astype(BF16))

        def nd_stage(g):
            phb = st['ph', g][3]
            nd = _nn(kvtz_s[g * 144:(g + 1) * 144, :], phb)
            rden = 1.0 / (nd[128:136, :] + DEN_EPS)
            o3 = nd[0:128, :].reshape(DH, 8, TS) * rden[None]
            dnum3 = doT_s[g * 128:(g + 1) * 128, tok].reshape(DH, 8, TS) * rden[None]
            st['dden', g] = -jnp.sum(dnum3 * o3, axis=0)
            st['dnum', g] = dnum3.reshape(128, TS).astype(BF16)
            st['o', g] = o3.reshape(128, TS)

        def bwd_stage(g):
            php, phm, ph, phb = st['ph', g]
            dnum = st['dnum', g]
            dden = st['dden', g]
            dph = _nn(kvm_s[g * 256:(g + 1) * 256, :], dnum)
            dkv_acc[g * 256:(g + 1) * 256, :] = jnp.where(i > 0, dkv_acc[g * 256:(g + 1) * 256, :], 0.0) + _nt(phb, dnum)
            zb = zb_s[g * 256:(g + 1) * 256, :]
            zbt = jnp.concatenate([zb] * (TS // 128), axis=1).reshape(2 * DH, 8, TS)
            dph3 = dph.reshape(2 * DH, 8, TS) + zbt * dden[None]
            dz_acc[g * 256:(g + 1) * 256, :] = jnp.where(i > 0, dz_acc[g * 256:(g + 1) * 256, :], 0.0) + _lane_fold(
                (ph.reshape(2 * DH, 8, TS) * dden[None]).reshape(256, TS))
            dp = _dual_softmax_bwd(php, phm, dph3[0:DH], dph3[DH:2 * DH])
            dpT_s[g * 128:(g + 1) * 128, tok] = dp.astype(BF16)

        def wn_chunk(j):
            rows = pl.ds(pl.multiple_of(j * 128, 128), 128)
            wN[:, rows] = wT[rows, :].astype(F32).T.astype(BF16)

        sm(0); fa(0); sm(1); fb(0)
        nd_stage(0); fc(0)
        bwd_stage(0); fa(1)
        nd_stage(1); sm(2); fb(1)
        bwd_stage(1); fc(1)
        nd_stage(2); sm(3); fa(2)
        bwd_stage(2); fb(2)
        nd_stage(3); fc(2)
        bwd_stage(3); fa(3)
        oT32 = jnp.concatenate([st['o', g] for g in range(NG)], axis=0)
        oT = oT32.astype(BF16)
        o = oT32.T.astype(BF16)
        fb(3); fc(3); fa(4)
        dyT = dy.astype(F32).T.astype(BF16)
        fb(4); fc(4); fa(5)
        wn_chunk(i)
        fb(5); fc(5); fa(6)
        wn_chunk(jnp.minimum(i + NTL, 3 * D // 128 - 1))
        fb(6); fc(6)
        nf = i > 0
        dwo_acc[...] = jnp.where(nf, dwo_acc[...], 0.0) + _nn(oT, dy)
        g_acc[:, 0:D] = jnp.where(nf, g_acc[:, 0:D], 0.0) + _nt(xnT, dpT_s[0:D, tok])
        y = x_v[tok, :].astype(F32) + _nn(o, wop[...]) + _nn(h_s[...], wd_v[...])
        o_out[tok, :] = y.astype(BF16)
        cp_out(i).start()
        dwdT_acc[...] = jnp.where(nf, dwdT_acc[...], 0.0) + _nn(dyT, h_s[...])
        dwgu_acc[...] = jnp.where(nf, dwgu_acc[...], 0.0) + _nn(xnT, dgu_s[tok, :])
        return carry

    with jax.named_scope("phase1"):
        jax.lax.fori_loop(0, NTL, phase1, 0)

    with jax.named_scope("prologue2"):
        hm = _head_mask()
        pi, pit = _perm_mats()
        for g in range(NG):
            rows = slice(g * 256, (g + 1) * 256)
            dkvm = _nn(jnp.where(hm, dkv_acc[rows, :], 0.0).astype(BF16), pi)
            kvm_s[rows, :] = dkvm.astype(BF16)
            kvtz_s[g * 144:g * 144 + 128, :] = dkvm.T.astype(BF16)
            zb_s[rows, :] = jnp.broadcast_to(jnp.sum(dz_acc[rows, :], axis=-1, keepdims=True), (256, 128))
        for g in range(NG):
            rows = slice(g * 128, (g + 1) * 128)
            o_dwo[rows, :] = _nn(pit, dwo_acc[rows, :].astype(BF16)).astype(BF16)
            gq = g_acc[:, rows].astype(BF16)
            o_dwqkv[:, rows] = _nn(gq, PT_s[rows, :]).astype(BF16)
            dP_s[:, rows] = _tn(wqkv_v[:, rows], gq)
        cp_dwo.start()
        cp_dwpart(0).start()

    def phase2(i, carry):
        tok = tile(i)
        KC = 2 * FF // NG
        dxn = None
        for g in range(NG):
            part = _nt(dgu_s[tok, g * KC:(g + 1) * KC], wgu_v[:, g * KC:(g + 1) * KC])
            dxn = part if dxn is None else dxn + part
            phb = phik_s[g * 256:(g + 1) * 256, tok]
            vT = vT_s[g * 128:(g + 1) * 128, tok]
            zb = zb_s[g * 256:(g + 1) * 256, :]
            zbt = jnp.concatenate([zb] * (TS // 128), axis=1)
            dph3 = (_nn(kvm_s[g * 256:(g + 1) * 256, :], vT) + zbt).reshape(2 * DH, 8, TS)
            dvT = _nn(kvtz_s[g * 144:g * 144 + 128, :], phb)
            ph3 = phb.astype(F32).reshape(2 * DH, 8, TS)
            dp = _dual_softmax_bwd(ph3[0:DH], ph3[DH:2 * DH], dph3[0:DH], dph3[DH:2 * DH])
            dpT_s[D + g * 128:D + (g + 1) * 128, tok] = dp.astype(BF16)
            dpT_s[2 * D + g * 128:2 * D + (g + 1) * 128, tok] = dvT.astype(BF16)
            if g == 0:
                o_dwg[piece(i), :] = dwgu_acc[piece(i), 0:FF].astype(BF16)
                o_dwu[piece(i), :] = dwgu_acc[piece(i), FF:2 * FF].astype(BF16)
            if g == 1:
                src = pl.ds(pl.multiple_of(jnp.minimum(i, NFC - 1) * FC, FC), FC)
                dst = pl.ds(pl.multiple_of(i * FC, FC), FC)
                o_dwd[dst, :] = dwdT_acc[:, src].T.astype(BF16)
        cp_dwg(i).start()
        cp_dwu(i).start()
        dxnT = _nn(wN[...], dpT_s[:, tok])
        g_acc[:, D:3 * D] = jnp.where(i > 0, g_acc[:, D:3 * D], 0.0) + _nt(xnT_s[:, tok], dpT_s[D:3 * D, tok])
        dxn = dxn + dxnT.T
        x = x_v[tok, :].astype(F32)
        mu = jnp.mean(x, axis=-1, keepdims=True)
        xc = x - mu
        var = jnp.mean(xc * xc, axis=-1, keepdims=True)
        rstd = jax.lax.rsqrt(var + LN_EPS)
        xn32 = xc * rstd
        m1 = jnp.mean(dxn, axis=-1, keepdims=True)
        m2 = jnp.mean(dxn * xn32, axis=-1, keepdims=True)
        dx = dy_v[tok, :].astype(F32) + rstd * (dxn - m1 - xn32 * m2)
        o_dx[tok, :] = dx.astype(BF16)
        cp_dx(i).start()

        @pl.when(i < NFC)
        def _():
            cp_dwd(i).start()

        return carry

    with jax.named_scope("phase2"):
        jax.lax.fori_loop(0, NTL, phase2, 0)

    with jax.named_scope("epilogue"):
        o_dwqkv[:, 2 * D:3 * D] = g_acc[:, 2 * D:3 * D].astype(BF16)
        cp_dwpart(2).start()
        gks = []
        for g in range(NG):
            kc = slice(D + g * 128, D + (g + 1) * 128)
            gk = g_acc[:, kc].astype(BF16)
            gks.append(gk)
            o_dwqkv[:, kc] = _nn(gk, PT_s[g * 128:(g + 1) * 128, :]).astype(BF16)
        cp_dwpart(1).start()
        sel, fmask, rep, hmask = _wphi_mats()
        dp_all = jnp.concatenate(
            [_tn(wqkv_v[:, D + g * 128:D + (g + 1) * 128], gks[g]) for g in range(NG)], axis=1) + dP_s[...]
        dpm = jnp.where(hmask, dp_all, 0.0).astype(BF16)
        t1 = jnp.where(fmask, _tn(rep, dpm), 0.0).astype(BF16)
        o_dwphi[...] = _nt(t1, sel).astype(BF16).reshape(DH, DH, H)
        cp_dwphi.start()
        for i in range(NTL):
            cp_out(i).wait()
            cp_dx(i).wait()
            cp_dwg(i).wait()
            cp_dwu(i).wait()
        for i in range(NFC):
            cp_dwd(i).wait()
        cp_dwo.wait()
        for part in range(3):
            cp_dwpart(part).wait()
        cp_dwphi.wait()


@jax.jit
def pallas_parallel_sum__linear_kernel_hedgehog__glu_gated_bilinear__prompt_kernel(
    A_x: jax.Array,
    A_wqkv: jax.Array,
    A_w_phi: jax.Array,
    A_wo: jax.Array,
    B_x: jax.Array,
    B_w_gate: jax.Array,
    B_w_up: jax.Array,
    B_w_down: jax.Array,
    grad_out: jax.Array,
):
    x2 = A_x.reshape(S, D)
    dy2 = grad_out.reshape(S, D)
    wphi_t = jnp.transpose(A_w_phi, (1, 2, 0))

    any_spec = pl.BlockSpec(memory_space=pl.ANY)
    out_shape = [
        jax.ShapeDtypeStruct((S, D), BF16),
        jax.ShapeDtypeStruct((S, D), BF16),
        jax.ShapeDtypeStruct((D, 3 * D), BF16),
        jax.ShapeDtypeStruct((DH, DH, H), BF16),
        jax.ShapeDtypeStruct((D, D), BF16),
        jax.ShapeDtypeStruct((D, FF), BF16),
        jax.ShapeDtypeStruct((D, FF), BF16),
        jax.ShapeDtypeStruct((FF, D), BF16),
    ]
    V = pltpu.VMEM
    DMA = pltpu.SemaphoreType.DMA
    scratch = [
        V((S, D), BF16), V((S, D), BF16), V((D, 3 * D), BF16), V((DH, DH, H), BF16), V((D, D), BF16),
        V((D, 2 * FF), BF16), V((FF, D), BF16),
        V((3 * D, D), BF16), V((D, 3 * D), BF16), V((D, D), BF16), V((D, 128), BF16), V((128, D), F32),
        V((S, D), BF16), V((D, S), BF16), V((2 * D, S), BF16), V((D, S), BF16), V((3 * D, S), BF16),
        V((D, S), F32), V((D, S), F32),
        V((2 * D, 128), F32), V((2 * D, 128), F32), V((2 * D, 128), F32), V((2 * D, 128), F32),
        V((2 * D, 128), BF16), V((NG * 144, 256), BF16), V((2 * D, 128), F32),
        V((TS, FF), BF16), V((S, 2 * FF), BF16),
        V((D, 3 * D), F32), V((D, D), F32), V((D, 2 * FF), F32), V((D, FF), F32),
        V((S, D), BF16), V((S, D), BF16), V((D, 3 * D), BF16), V((DH, DH, H), BF16), V((D, D), BF16),
        V((D, FF), BF16), V((D, FF), BF16), V((NTL * FC, D), BF16),
        DMA((NTL,)), DMA((NTL,)), DMA((8,)), DMA((NTL,)), DMA((NTL,)), DMA((5,)),
        DMA((NTL,)), DMA((NTL,)), DMA((NFC,)),
    ]
    outs = pl.pallas_call(
        _kernel,
        in_specs=[any_spec] * 8,
        out_specs=[any_spec] * 8,
        out_shape=out_shape,
        scratch_shapes=scratch,
        compiler_params=pltpu.CompilerParams(vmem_limit_bytes=110 * 1024 * 1024),
    )(x2, dy2, A_wqkv, wphi_t, A_wo, B_w_gate, B_w_up, B_w_down)
    out, dx, dwqkv, dwphi_t, dwo, dwg, dwu, dwd = outs
    return (out.reshape(1, S, D), dx.reshape(1, S, D), dwqkv, jnp.transpose(dwphi_t, (2, 0, 1)),
            dwo, dwg, dwu, dwd)
```

```python
import jax
import jax.numpy as jnp
import jax.experimental.pallas as pl
import jax.experimental.pallas.tpu as pltpu

F32 = jnp.float32
BF16 = jnp.bfloat16

S = 2048
D = 512
H = 32
DH = 16
FF = 1792
NG = 4
TS = 256
NTL = S // TS
FC = 256
NFC = FF // FC
RP = D // NTL
ORDER1 = "F s0 F n0 F F b0 F s1 F n1 F F b1 F s2 F n2 F F b2 F s3 F n3 F b3 to ty w0 w1"
ORDER0 = "k0 k1 s0 v s1 k2 a0 a1 q0 s2 k3 q1 a2 q2 s3 do a3 ln q3"
LN_EPS = 1e-5
DEN_EPS = 1e-6


def _nn(a, b):
    return jnp.dot(a, b, preferred_element_type=F32)


def _nt(a, b):
    return jax.lax.dot_general(a, b, (((1,), (1,)), ((), ())), preferred_element_type=F32)


def _tn(a, b):
    return jax.lax.dot_general(a, b, (((0,), (0,)), ((), ())), preferred_element_type=F32)


def _iota(shape, dim):
    return jax.lax.broadcasted_iota(jnp.int32, shape, dim)


def _onehot(cond):
    return jnp.where(cond, 1.0, 0.0).astype(BF16)


def _dual_softmax(p):
    t = p.shape[-1]
    p3 = p.reshape(DH, 8, t)
    mx = jnp.max(p3, axis=0)
    mn = jnp.min(p3, axis=0)
    ep = jnp.exp(p3 - mx[None])
    em = jnp.exp(mn[None] - p3)
    rp = 1.0 / jnp.sum(ep, axis=0)
    rm = 1.0 / jnp.sum(em, axis=0)
    return ep * rp[None], em * rm[None]


def _dual_softmax_bwd(php, phm, dphp, dphm):
    tp = jnp.sum(dphp * php, axis=0)
    tm = jnp.sum(dphm * phm, axis=0)
    dp = php * (dphp - tp[None]) - phm * (dphm - tm[None])
    return dp.reshape(128, dp.shape[-1])


def _lane_fold(a):
    t = a.shape[-1]
    acc = a[:, 0:128]
    for j in range(1, t // 128):
        acc = acc + a[:, j * 128:(j + 1) * 128]
    return acc


def _perm_mats():
    r = _iota((128, 128), 0)
    c = _iota((128, 128), 1)
    pi = _onehot((r // 8 == c % 16) & (r % 8 == c // 16))
    pit = _onehot((c // 8 == r % 16) & (c % 8 == r // 16))
    return pi, pit


def _wphi_mats():
    h = _iota((H, D), 0)
    j = _iota((H, D), 1)
    sel = _onehot(h == (j // 128) * 8 + j % 8)
    a = _iota((256, D), 0)
    j2 = _iota((256, D), 1)
    fmask = a % 16 == (j2 % 128) // 8
    c = _iota((128, 256), 0)
    a2 = _iota((128, 256), 1)
    rep = _onehot(c % 16 == a2 // 16)
    c3 = _iota((128, D), 0)
    j3 = _iota((128, D), 1)
    hmask = c3 // 16 == j3 % 8
    return sel, fmask, rep, hmask


def _head_mask():
    r = _iota((256, 128), 0)
    c = _iota((256, 128), 1)
    return r % 8 == c % 8


def _kernel(x_hbm, dy_hbm, wqkv_hbm, wphi_hbm, wo_hbm, wg_hbm, wu_hbm, wd_hbm,
            out_hbm, dx_hbm, dwqkv_hbm, dwphi_hbm, dwo_hbm, dwg_hbm, dwu_hbm, dwd_hbm,
            x_v, dy_v, wqkv_v, wphi_v, wo_v, wgu_v, wd_v,
            wT, wN, wop, PT_s, dP_s,
            xn_s, xnT_s, phik_s, vT_s, dpT_s, pq_s, doT_s, rstd_s,
            kv_acc, z_acc, dkv_acc, dz_acc,
            kvm_s, kvtz_s, zb_s,
            h_s, dgu_s,
            g_acc, dwo_acc, dwgu_acc, dwdT_acc,
            o_out, o_dx, o_dwqkv, o_dwphi, o_dwo, o_dwg, o_dwu, o_dwd,
            sem_x, sem_dy, sem_w, sem_o, sem_dx, sem_dw, sem_g, sem_u, sem_d):

    def tile(i):
        return pl.ds(pl.multiple_of(i * TS, TS), TS)

    def cp_x(i):
        return pltpu.make_async_copy(x_hbm.at[tile(jnp.minimum(i, NTL - 1)), :], x_v.at[tile(i), :], sem_x.at[i])

    def cp_dy(i):
        return pltpu.make_async_copy(dy_hbm.at[tile(i), :], dy_v.at[tile(i), :], sem_dy.at[i])

    def cp_out(i):
        return pltpu.make_async_copy(o_out.at[tile(i), :], out_hbm.at[tile(i), :], sem_o.at[i])

    def cp_dx(i):
        return pltpu.make_async_copy(o_dx.at[tile(i), :], dx_hbm.at[tile(i), :], sem_dx.at[i])

    def piece(i):
        return pl.ds(pl.multiple_of(i * RP, RP), RP)

    def cp_dwg(i):
        return pltpu.make_async_copy(o_dwg.at[piece(i), :], dwg_hbm.at[piece(i), :], sem_g.at[i])

    def cp_dwu(i):
        return pltpu.make_async_copy(o_dwu.at[piece(i), :], dwu_hbm.at[piece(i), :], sem_u.at[i])

    def cp_dwd(i):
        rows = pl.ds(pl.multiple_of(i * FC, FC), FC)
        return pltpu.make_async_copy(o_dwd.at[rows, :], dwd_hbm.at[rows, :], sem_d.at[i])

    def cp_wpart(part):
        cols = slice(part * D, (part + 1) * D)
        return pltpu.make_async_copy(wqkv_hbm.at[:, cols], wqkv_v.at[:, cols], sem_w.at[part])

    def cp_dwpart(part):
        cols = slice(part * D, (part + 1) * D)
        return pltpu.make_async_copy(o_dwqkv.at[:, cols], dwqkv_hbm.at[:, cols], sem_dw.at[part])

    cp_wphi = pltpu.make_async_copy(wphi_hbm, wphi_v, sem_w.at[3])
    cp_wo = pltpu.make_async_copy(wo_hbm, wo_v, sem_w.at[4])
    cp_wg = pltpu.make_async_copy(wg_hbm, wgu_v.at[:, 0:FF], sem_w.at[5])
    cp_wu = pltpu.make_async_copy(wu_hbm, wgu_v.at[:, FF:2 * FF], sem_w.at[6])
    cp_wd = pltpu.make_async_copy(wd_hbm, wd_v, sem_w.at[7])
    cp_dwphi = pltpu.make_async_copy(o_dwphi, dwphi_hbm, sem_dw.at[3])
    cp_dwo = pltpu.make_async_copy(o_dwo, dwo_hbm, sem_dw.at[4])

    def layernorm_tile(j):
        tok = tile(j)
        x = x_v[tok, :].astype(F32)
        mu = jnp.mean(x, axis=-1, keepdims=True)
        xc = x - mu
        var = jnp.mean(xc * xc, axis=-1, keepdims=True)
        rstd = jax.lax.rsqrt(var + LN_EPS)
        xn32 = xc * rstd
        rstd_s[tok, :] = jnp.broadcast_to(rstd, (TS, 128))
        xn_s[tok, :] = xn32.astype(BF16)
        xnT_s[:, tok] = xn32.T.astype(BF16)

    def phase0_step(i, first):
        tok = tile(i)
        st = {}
        xn = xn_s[tok, :]

        def acc(ref, rows, val):
            ref[rows, :] = val if first else ref[rows, :] + val

        def pkm(g):
            st['pk', g] = _nt(wT[D + g * 128:D + (g + 1) * 128, :], xn)

        def sm(g):
            php, phm = _dual_softmax(st['pk', g])
            ph = jnp.concatenate([php.reshape(128, TS), phm.reshape(128, TS)], axis=0)
            phb = ph.astype(BF16)
            phik_s[g * 256:(g + 1) * 256, tok] = phb
            acc(z_acc, slice(g * 256, (g + 1) * 256), _lane_fold(ph))
            st[g] = phb

        def vm():
            vT = _nt(wT[2 * D:3 * D, :], xn).astype(BF16)
            vT_s[:, tok] = vT
            st['v'] = vT

        def pqm(g):
            pq_s[g * 128:(g + 1) * 128, tok] = _nt(wT[g * 128:(g + 1) * 128, :], xn)

        def kvm(g):
            acc(kv_acc, slice(g * 256, (g + 1) * 256), _nt(st[g], st['v'][g * 128:(g + 1) * 128, :]))

        def dom():
            doT_s[:, tok] = _nt(wop[...], dy_v[tok, :])

        return pkm, sm, vm, pqm, kvm, dom

    with jax.named_scope("prologue"):
        cp_wphi.start()
        cp_x(0).start()
        cp_wpart(1).start()
        sel, fmask, rep, hmask = _wphi_mats()
        cp_wphi.wait()
        a2 = wphi_v[...].reshape(DH * DH, H)
        b = jnp.where(fmask, _nn(a2, sel), 0.0).astype(BF16)
        p_all = jnp.where(hmask, _nn(rep, b), 0.0)
        for g in range(NG):
            PT_s[g * 128:(g + 1) * 128, :] = p_all[:, g * 128:(g + 1) * 128].T.astype(BF16)

        def prep(part):
            for g in range(NG):
                cols = slice(part * D + g * 128, part * D + (g + 1) * 128)
                wT[cols, :] = _nt(PT_s[g * 128:(g + 1) * 128, :], wqkv_v[:, cols]).astype(BF16)

        cp_x(0).wait()
        cp_wpart(2).start()
        cp_wpart(1).wait()
        cp_wpart(0).start()
        prep(1)
        layernorm_tile(0)
        pkm, sm, vm, pqm, kvm, dom = phase0_step(0, True)
        pkm(0); pkm(1); sm(0); pkm(2); sm(1); pkm(3); sm(2); sm(3)
        cp_wpart(2).wait()
        cp_wo.start()
        cp_dy(0).start()
        cp_x(1).start()
        cp_wpart(0).wait()
        prep(0)
        wT[2 * D:3 * D, :] = wqkv_v[:, 2 * D:3 * D].astype(F32).T.astype(BF16)
        pqm(0)
        vm()
        pqm(1)
        kvm(0); kvm(1); kvm(2); kvm(3)
        pqm(2); pqm(3)
        cp_wo.wait()
        cp_dy(0).wait()
        cp_x(1).wait()
        cp_x(2).start()
        cp_dy(1).start()
        pi, _ = _perm_mats()
        for g in range(NG):
            rows = slice(g * 128, (g + 1) * 128)
            wop[rows, :] = _nn(pi, wo_v[rows, :]).astype(BF16)
        layernorm_tile(1)
        dom()

    def phase0(i, carry):
        cp_x(i + 1).wait()
        cp_dy(i).wait()

        @pl.when(i + 1 < NTL)
        def _():
            cp_x(i + 2).start()
            cp_dy(i + 1).start()

        @pl.when(i == 1)
        def _():
            cp_wd.start()

        @pl.when(i == 2)
        def _():
            cp_wg.start()

        @pl.when(i == 3)
        def _():
            cp_wu.start()

        pkm, sm, vm, pqm, kvm, dom = phase0_step(i, False)
        for tokn in ORDER0.split():
            if tokn == 'v':
                vm()
            elif tokn == 'do':
                dom()
            elif tokn == 'ln':
                layernorm_tile(jnp.minimum(i + 1, NTL - 1))
            else:
                {'k': pkm, 's': sm, 'q': pqm, 'a': kvm}[tokn[0]](int(tokn[1]))
        return carry

    with jax.named_scope("phase0"):
        jax.lax.fori_loop(1, NTL, phase0, 0)

    with jax.named_scope("prologue1"):
        r = _iota((256, 128), 0)
        c = _iota((256, 128), 1)
        eye16 = _onehot(_iota((16, 128), 0) == _iota((16, 128), 1))
        pi, pit = _perm_mats()
        for g in range(NG):
            rows = slice(g * 256, (g + 1) * 256)
            kvn = jnp.where(r % 8 == c // 16, kv_acc[rows, :], 0.0).astype(BF16)
            kvm = _nn(kvn, pit)
            zb = jnp.broadcast_to(jnp.sum(z_acc[rows, :], axis=-1, keepdims=True), (256, 128))
            zb_s[rows, :] = zb
            zc = jnp.where(c == r % 8, zb, 0.0)
            kvm_s[rows, :] = kvm.astype(BF16)
            kvtz_s[g * 144:g * 144 + 128, :] = _nt(pi, kvn).astype(BF16)
            kvtz_s[g * 144 + 128:(g + 1) * 144, :] = _nt(eye16, zc.astype(BF16)).astype(BF16)
        cp_wd.wait()
        cp_wg.wait()
        cp_wu.wait()

    def phase1(i, carry):
        tok = tile(i)
        xn = xn_s[tok, :]
        xnT = xnT_s[:, tok]
        dy = dy_v[tok, :]
        st = {}

        def fa(c):
            st['gg', c] = _nn(xn, wgu_v[:, c * FC:(c + 1) * FC])

        def fb(c):
            uu = _nn(xn, wgu_v[:, FF + c * FC:FF + (c + 1) * FC])
            st['uu', c] = uu
            h_s[:, c * FC:(c + 1) * FC] = (st['gg', c] * uu).astype(BF16)

        def fc(c):
            dh = _nt(dy, wd_v[c * FC:(c + 1) * FC, :])
            dgu_s[tok, c * FC:(c + 1) * FC] = (dh * st['uu', c]).astype(BF16)
            dgu_s[tok, FF + c * FC:FF + (c + 1) * FC] = (dh * st['gg', c]).astype(BF16)

        def sm(g):
            php, phm = _dual_softmax(pq_s[g * 128:(g + 1) * 128, tok])
            ph = jnp.concatenate([php.reshape(128, TS), phm.reshape(128, TS)], axis=0)
            st['ph', g] = (php, phm, ph, ph.astype(BF16))

        def nd_stage(g):
            phb = st['ph', g][3]
            nd = _nn(kvtz_s[g * 144:(g + 1) * 144, :], phb)
            rden = 1.0 / (nd[128:136, :] + DEN_EPS)
            o3 = nd[0:128, :].reshape(DH, 8, TS) * rden[None]
            dnum3 = doT_s[g * 128:(g + 1) * 128, tok].reshape(DH, 8, TS) * rden[None]
            st['dden', g] = -jnp.sum(dnum3 * o3, axis=0)
            st['dnum', g] = dnum3.reshape(128, TS).astype(BF16)
            st['o', g] = o3.reshape(128, TS)

        def bwd_stage(g):
            php, phm, ph, phb = st['ph', g]
            dnum = st['dnum', g]
            dden = st['dden', g]
            dph = _nn(kvm_s[g * 256:(g + 1) * 256, :], dnum)
            dkv_acc[g * 256:(g + 1) * 256, :] = jnp.where(i > 0, dkv_acc[g * 256:(g + 1) * 256, :], 0.0) + _nt(phb, dnum)
            zb = zb_s[g * 256:(g + 1) * 256, :]
            zbt = jnp.concatenate([zb] * (TS // 128), axis=1).reshape(2 * DH, 8, TS)
            dph3 = dph.reshape(2 * DH, 8, TS) + zbt * dden[None]
            dz_acc[g * 256:(g + 1) * 256, :] = jnp.where(i > 0, dz_acc[g * 256:(g + 1) * 256, :], 0.0) + _lane_fold(
                (ph.reshape(2 * DH, 8, TS) * dden[None]).reshape(256, TS))
            dp = _dual_softmax_bwd(php, phm, dph3[0:DH], dph3[DH:2 * DH])
            dpT_s[g * 128:(g + 1) * 128, tok] = dp.astype(BF16)

        def wn_chunk(j):
            rows = pl.ds(pl.multiple_of(j * 128, 128), 128)
            wN[:, rows] = wT[rows, :].astype(F32).T.astype(BF16)

        def tr_o():
            oT32 = jnp.concatenate([st['o', g] for g in range(NG)], axis=0)
            st['oT'] = oT32.astype(BF16)
            st['oN'] = oT32.T.astype(BF16)

        def tr_dy():
            st['dyT'] = dy.astype(F32).T.astype(BF16)

        fillers = [(f, c) for c in range(NFC) for f in (fa, fb, fc)]
        table = {'s': sm, 'n': nd_stage, 'b': bwd_stage}
        for tokn in ORDER1.split():
            if tokn == 'F':
                f, c = fillers.pop(0)
                f(c)
            elif tokn == 'to':
                tr_o()
            elif tokn == 'ty':
                tr_dy()
            elif tokn == 'w0':
                wn_chunk(i)
            elif tokn == 'w1':
                wn_chunk(jnp.minimum(i + NTL, 3 * D // 128 - 1))
            else:
                table[tokn[0]](int(tokn[1]))
        for f, c in fillers:
            f(c)
        oT, o, dyT = st['oT'], st['oN'], st['dyT']
        nf = i > 0
        dwo_acc[...] = jnp.where(nf, dwo_acc[...], 0.0) + _nn(oT, dy)
        g_acc[:, 0:D] = jnp.where(nf, g_acc[:, 0:D], 0.0) + _nt(xnT, dpT_s[0:D, tok])
        y = x_v[tok, :].astype(F32) + _nn(o, wop[...]) + _nn(h_s[...], wd_v[...])
        o_out[tok, :] = y.astype(BF16)
        cp_out(i).start()
        dwdT_acc[...] = jnp.where(nf, dwdT_acc[...], 0.0) + _nn(dyT, h_s[...])
        dwgu_acc[...] = jnp.where(nf, dwgu_acc[...], 0.0) + _nn(xnT, dgu_s[tok, :])
        return carry

    with jax.named_scope("phase1"):
        jax.lax.fori_loop(0, NTL, phase1, 0)

    with jax.named_scope("prologue2"):
        hm = _head_mask()
        pi, pit = _perm_mats()
        for g in range(NG):
            rows = slice(g * 256, (g + 1) * 256)
            dkvm = _nn(jnp.where(hm, dkv_acc[rows, :], 0.0).astype(BF16), pi)
            kvm_s[rows, :] = dkvm.astype(BF16)
            kvtz_s[g * 144:g * 144 + 128, :] = dkvm.T.astype(BF16)
            zb_s[rows, :] = jnp.broadcast_to(jnp.sum(dz_acc[rows, :], axis=-1, keepdims=True), (256, 128))
        for g in range(NG):
            rows = slice(g * 128, (g + 1) * 128)
            o_dwo[rows, :] = _nn(pit, dwo_acc[rows, :].astype(BF16)).astype(BF16)
            gq = g_acc[:, rows].astype(BF16)
            o_dwqkv[:, rows] = _nn(gq, PT_s[rows, :]).astype(BF16)
            dP_s[:, rows] = _tn(wqkv_v[:, rows], gq)
        o_dwg[piece(NTL - 1), :] = dwgu_acc[piece(NTL - 1), 0:FF].astype(BF16)
        o_dwu[piece(NTL - 1), :] = dwgu_acc[piece(NTL - 1), FF:2 * FF].astype(BF16)
        cp_dwg(NTL - 1).start()
        cp_dwu(NTL - 1).start()
        cp_dwo.start()
        cp_dwpart(0).start()

    def phase2(i, carry):
        tok = tile(i)
        KC = 2 * FF // NG
        dxn = None
        for g in range(NG):
            part = _nt(dgu_s[tok, g * KC:(g + 1) * KC], wgu_v[:, g * KC:(g + 1) * KC])
            dxn = part if dxn is None else dxn + part
            phb = phik_s[g * 256:(g + 1) * 256, tok]
            vT = vT_s[g * 128:(g + 1) * 128, tok]
            zb = zb_s[g * 256:(g + 1) * 256, :]
            zbt = jnp.concatenate([zb] * (TS // 128), axis=1)
            dph3 = (_nn(kvm_s[g * 256:(g + 1) * 256, :], vT) + zbt).reshape(2 * DH, 8, TS)
            dvT = _nn(kvtz_s[g * 144:g * 144 + 128, :], phb)
            ph3 = phb.astype(F32).reshape(2 * DH, 8, TS)
            dp = _dual_softmax_bwd(ph3[0:DH], ph3[DH:2 * DH], dph3[0:DH], dph3[DH:2 * DH])
            dpT_s[D + g * 128:D + (g + 1) * 128, tok] = dp.astype(BF16)
            dpT_s[2 * D + g * 128:2 * D + (g + 1) * 128, tok] = dvT.astype(BF16)
            if g == 0:
                psrc = piece(jnp.minimum(i, NTL - 2))
                pdst = piece(i + i // (NTL - 1))
                o_dwg[pdst, :] = dwgu_acc[psrc, 0:FF].astype(BF16)
                o_dwu[pdst, :] = dwgu_acc[psrc, FF:2 * FF].astype(BF16)
            if g == 1:
                src = pl.ds(pl.multiple_of(jnp.minimum(i, NFC - 1) * FC, FC), FC)
                dst = pl.ds(pl.multiple_of(i * FC, FC), FC)
                o_dwd[dst, :] = dwdT_acc[:, src].T.astype(BF16)
        dxnT = _nn(wN[...], dpT_s[:, tok])
        g_acc[:, D:3 * D] = jnp.where(i > 0, g_acc[:, D:3 * D], 0.0) + _nt(xnT_s[:, tok], dpT_s[D:3 * D, tok])
        dxn = dxn + dxnT.T
        rstd = jnp.concatenate([rstd_s[tok, :]] * (D // 128), axis=1)
        xn32 = xn_s[tok, :].astype(F32)
        m1 = jnp.mean(dxn, axis=-1, keepdims=True)
        m2 = jnp.mean(dxn * xn32, axis=-1, keepdims=True)
        dx = dy_v[tok, :].astype(F32) + rstd * (dxn - m1 - xn32 * m2)
        o_dx[tok, :] = dx.astype(BF16)
        cp_dx(i).start()

        @pl.when(i < NTL - 1)
        def _():
            cp_dwg(i).start()
            cp_dwu(i).start()
            cp_dwd(i).start()

        return carry

    with jax.named_scope("phase2"):
        jax.lax.fori_loop(0, NTL, phase2, 0)

    with jax.named_scope("epilogue"):
        o_dwqkv[:, 2 * D:3 * D] = g_acc[:, 2 * D:3 * D].astype(BF16)
        cp_dwpart(2).start()
        gks = []
        for g in range(NG):
            kc = slice(D + g * 128, D + (g + 1) * 128)
            gk = g_acc[:, kc].astype(BF16)
            gks.append(gk)
            o_dwqkv[:, kc] = _nn(gk, PT_s[g * 128:(g + 1) * 128, :]).astype(BF16)
        cp_dwpart(1).start()
        sel, fmask, rep, hmask = _wphi_mats()
        dp_all = jnp.concatenate(
            [_tn(wqkv_v[:, D + g * 128:D + (g + 1) * 128], gks[g]) for g in range(NG)], axis=1) + dP_s[...]
        dpm = jnp.where(hmask, dp_all, 0.0).astype(BF16)
        t1 = jnp.where(fmask, _tn(rep, dpm), 0.0).astype(BF16)
        o_dwphi[...] = _nt(t1, sel).astype(BF16).reshape(DH, DH, H)
        cp_dwphi.start()
        for i in range(NTL):
            cp_out(i).wait()
            cp_dx(i).wait()
            cp_dwg(i).wait()
            cp_dwu(i).wait()
        for i in range(NFC):
            cp_dwd(i).wait()
        cp_dwo.wait()
        for part in range(3):
            cp_dwpart(part).wait()
        cp_dwphi.wait()


@jax.jit
def pallas_parallel_sum__linear_kernel_hedgehog__glu_gated_bilinear__prompt_kernel(
    A_x: jax.Array,
    A_wqkv: jax.Array,
    A_w_phi: jax.Array,
    A_wo: jax.Array,
    B_x: jax.Array,
    B_w_gate: jax.Array,
    B_w_up: jax.Array,
    B_w_down: jax.Array,
    grad_out: jax.Array,
):
    x2 = A_x.reshape(S, D)
    dy2 = grad_out.reshape(S, D)
    wphi_t = jnp.transpose(A_w_phi, (1, 2, 0))

    any_spec = pl.BlockSpec(memory_space=pl.ANY)
    out_shape = [
        jax.ShapeDtypeStruct((S, D), BF16),
        jax.ShapeDtypeStruct((S, D), BF16),
        jax.ShapeDtypeStruct((D, 3 * D), BF16),
        jax.ShapeDtypeStruct((DH, DH, H), BF16),
        jax.ShapeDtypeStruct((D, D), BF16),
        jax.ShapeDtypeStruct((D, FF), BF16),
        jax.ShapeDtypeStruct((D, FF), BF16),
        jax.ShapeDtypeStruct((FF, D), BF16),
    ]
    V = pltpu.VMEM
    DMA = pltpu.SemaphoreType.DMA
    scratch = [
        V((S + TS, D), BF16), V((S, D), BF16), V((D, 3 * D), BF16), V((DH, DH, H), BF16), V((D, D), BF16),
        V((D, 2 * FF), BF16), V((FF, D), BF16),
        V((3 * D, D), BF16), V((D, 3 * D), BF16), V((D, D), BF16), V((D, 128), BF16), V((128, D), F32),
        V((S, D), BF16), V((D, S), BF16), V((2 * D, S), BF16), V((D, S), BF16), V((3 * D, S), BF16),
        V((D, S), F32), V((D, S), F32), V((S, 128), F32),
        V((2 * D, 128), F32), V((2 * D, 128), F32), V((2 * D, 128), F32), V((2 * D, 128), F32),
        V((2 * D, 128), BF16), V((NG * 144, 256), BF16), V((2 * D, 128), F32),
        V((TS, FF), BF16), V((S, 2 * FF), BF16),
        V((D, 3 * D), F32), V((D, D), F32), V((D, 2 * FF), F32), V((D, FF), F32),
        V((S, D), BF16), V((S, D), BF16), V((D, 3 * D), BF16), V((DH, DH, H), BF16), V((D, D), BF16),
        V((D + RP, FF), BF16), V((D + RP, FF), BF16), V((NTL * FC, D), BF16),
        DMA((NTL + 1,)), DMA((NTL,)), DMA((8,)), DMA((NTL,)), DMA((NTL,)), DMA((5,)),
        DMA((NTL,)), DMA((NTL,)), DMA((NTL,)),
    ]
    outs = pl.pallas_call(
        _kernel,
        in_specs=[any_spec] * 8,
        out_specs=[any_spec] * 8,
        out_shape=out_shape,
        scratch_shapes=scratch,
        compiler_params=pltpu.CompilerParams(vmem_limit_bytes=110 * 1024 * 1024),
    )(x2, dy2, A_wqkv, wphi_t, A_wo, B_w_gate, B_w_up, B_w_down)
    out, dx, dwqkv, dwphi_t, dwo, dwg, dwu, dwd = outs
    return (out.reshape(1, S, D), dx.reshape(1, S, D), dwqkv, jnp.transpose(dwphi_t, (2, 0, 1)),
            dwo, dwg, dwu, dwd)
```
